```python
import jax
import jax.numpy as jnp

def _softmax(x, axis=-1):
    return jax.nn.softmax(x, axis=axis)
def _gelu(x):
    return jax.nn.gelu(x, approximate=True)
def _silu(x):
    return jax.nn.silu(x)
def _sigmoid(x):
    return jax.nn.sigmoid(x)
def _layernorm(x, axis=-1, eps=1e-5):
    m = jnp.mean(x, axis=axis, keepdims=True)
    v = jnp.var(x, axis=axis, keepdims=True)
    return (x - m) / jnp.sqrt(v + eps)
def _scatter_add(tgt, idx, src, axis=0):
    return tgt.at[idx].add(src)
def _segment_sum(src, seg, n):
    return jax.ops.segment_sum(src, seg, n)
class _Rng:
    def __init__(self, key):
        self._k = key
    def _next(self):
        self._k, sub = jax.random.split(self._k)
        return sub
    def normal(self, shape):
        return jax.random.normal(self._next(), shape, dtype=jnp.bfloat16)
    def randint(self, lo, hi, shape):
        return jax.random.randint(self._next(), shape, lo, hi, dtype=jnp.int32)
    def uniform(self, shape, lo=0.0, hi=1.0):
        return jax.random.uniform(self._next(), shape, jnp.bfloat16, lo, hi)
    def permutation(self, n):
        return jax.random.permutation(self._next(), n)


kernel_name = 'standalone__winograd__vision'

def setup_inputs():
    _rng = _Rng(jax.random.key(int.from_bytes(__import__("os").urandom(4), "little")))
    _w = (lambda a: (lambda t: t.astype(jnp.bfloat16) if jnp.issubdtype(t.dtype, jnp.floating) else t)(jnp.asarray(a)))
    H = W = 512 // 2 * 2
    C = 192
    return {
        "x": _w((lambda *s: _rng.normal(s) * 0.05)(1, H, W, C)),
        "w": _w((lambda *s: _rng.normal(s) * 0.05)(3, 3, C, C)),
    }

def reference(x, w):
    N, H, W, C = x.shape
    K = w.shape[-1]
    G  = jnp.array([[1.0,0.0,0.0],[0.5,0.5,0.5],[0.5,-0.5,0.5],[0.0,0.0,1.0]], dtype=x.dtype)
    Bt = jnp.array([[1.0,0.0,-1.0,0.0],[0.0,1.0,1.0,0.0],[0.0,-1.0,1.0,0.0],[0.0,1.0,0.0,-1.0]], dtype=x.dtype)
    At = jnp.array([[1.0,1.0,1.0,0.0],[0.0,1.0,-1.0,-1.0]], dtype=x.dtype)
    U = jnp.einsum("ar,rsck,bs->abck", G, w, G)
    xp = jnp.pad(x, ((0,0),(1,1),(1,1),(0,0)))
    nH, nW = H // 2, W // 2
    patches = []
    for i in range(4):
        for j in range(4):
            patches.append(xp[:, i:i + 2 * nH:2, j:j + 2 * nW:2, :])
    d = jnp.stack(patches).reshape(4, 4, N * nH * nW, C)
    V = jnp.einsum("ai,ijpc,bj->abpc", Bt, d, Bt)
    M = jnp.einsum("abck,abpc->abpk", U, V)
    Y = jnp.einsum("ma,abpk,nb->pmnk", At, M, At)
    Y = Y.reshape(N, nH, nW, 2, 2, K)
    Y = (lambda x, *d: x.transpose(*d))(Y, 0, 1, 3, 2, 4, 5).reshape(N, H, W, K)
    return Y
```

```python
import numpy as np
import jax
import jax.numpy as jnp
import jax.experimental.pallas as pl
import jax.experimental.pallas.tpu as pltpu

PA, PB = 0.7, 1.425
_pts = [0.0, PA, -PA, PB, -PB]
GH = np.zeros((6, 3))
for _i, _p in enumerate(_pts):
    GH[_i] = np.array([1.0, _p, _p * _p]) / np.prod([_p - q for q in _pts if q != _p])
GH[5, 2] = 1.0
GW = np.array([[1.0, 0, 0], [0.5, 0.5, 0.5], [0.5, -0.5, 0.5], [0, 0, 1.0]])
A2, B2 = PA * PA, PB * PB
F32, BF16, U32 = jnp.float32, jnp.bfloat16, jnp.uint32
C = 192
W = 512
P = W // 2


def _dot(a, b):
    return jnp.dot(a, b, preferred_element_type=F32)


def _kernel(x_hbm, w_ref, o_ref, xb, sem, ut, wr, vm, vr, ys):
    i = pl.program_id(0)
    n = pl.num_programs(0)
    H = x_hbm.shape[0]

    def full_copy(j, s):
        return pltpu.make_async_copy(x_hbm.at[pl.ds(8 * j + 5, 8)], xb.at[s], sem.at[s])

    def last_copy(s):
        return pltpu.make_async_copy(x_hbm.at[pl.ds(H - 3, 3)], xb.at[s, pl.ds(0, 3)], sem.at[s])

    lane = jax.lax.broadcasted_iota(jnp.int32, (96, 128), 1)
    lo = lane < 64
    idx_de = jnp.where(lo, 2 * lane, 2 * lane - 127)
    idx_in = (lane >> 1) + 64 * (lane & 1)
    zero = jnp.zeros((96, 128), U32)
    f32 = lambda u: pltpu.bitcast(u, BF16).astype(F32)

    def wstage(s, slot):
        if True:
            g = [jnp.take_along_axis(
                pltpu.bitcast(xb[s, slot, :, 128 * j:128 * j + 128], U32), idx_de, axis=1)
                for j in range(4)]
            r = [pltpu.roll(t, 64, 1) for t in g]
            E = [jnp.where(lo, g[2 * q], r[2 * q + 1]) for q in range(2)]
            O = [jnp.where(lo, r[2 * q], g[2 * q + 1]) for q in range(2)]
            Or = [pltpu.roll(t, 1, 1) for t in O]
            Er = [pltpu.roll(t, 127, 1) for t in E]
            Os = [jnp.where(lane == 0, zero, Or[0]), jnp.where(lane == 0, Or[0], Or[1])]
            Es = [jnp.where(lane == 127, Er[1], Er[0]), jnp.where(lane == 127, zero, Er[1])]
            for q in range(2):
                e, o = f32(E[q]), f32(O[q])
                sl = (slice(None), slice(128 * q, 128 * q + 128))
                wr[(slot, 0) + sl] = f32(Os[q]) - o
                wr[(slot, 1) + sl] = e + o
                wr[(slot, 2) + sl] = o - e
                wr[(slot, 3) + sl] = e - f32(Es[q])

    remoff = {0: 0, 1: 64, 3: 128, 2: 192}

    def hstage(par, slots, b):
        for c in range(0, C, 16):
            for q in range(2):
                ls = slice(128 * q, 128 * q + 128)
                d = [wr[sl, b, c:c + 16, ls] for sl in slots]
                t1 = d[4] - B2 * d[2]
                t2 = PA * d[3] - (PA * B2) * d[1]
                t3 = d[4] - A2 * d[2]
                t4 = PB * d[3] - (PB * A2) * d[1]
                v = [(d[4] + (A2 * B2) * d[0]) - (A2 + B2) * d[2], t1 + t2, t1 - t2, t3 + t4, t3 - t4,
                     (d[5] + (A2 * B2) * d[1]) - (A2 + B2) * d[3]]
                for a in range(6):
                    if c < 128:
                        vm[par, a, b, c:c + 16, ls] = v[a].astype(BF16)
                    else:
                        r0 = remoff[b] + c - 128
                        vr[par, a, r0:r0 + 16, ls] = v[a].astype(BF16)

    def mm(par, a):
        m1 = _dot(ut[a, 1], vm[par, a, 1])
        m2 = _dot(ut[a, 2], vm[par, a, 2]) + _dot(ut[a, 6][:, :64], vr[par, a, 192:256])
        ye = _dot(ut[a, 0], vm[par, a, 0]) + _dot(ut[a, 4], vr[par, a, 0:128])
        ys[par, a, 0] = (m1 + m2) + ye
        yo = _dot(ut[a, 3], vm[par, a, 3]) + _dot(ut[a, 5], vr[par, a, 64:192])
        ys[par, a, 1] = (m1 - m2) + yo

    def ostage(par):
        if True:
            for q in range(2):
                y = []
                for e in range(2):
                    m = [ys[par, a, e, :, 128 * q:128 * q + 128] for a in range(6)]
                    s1, d1, s2, d2 = m[1] + m[2], m[1] - m[2], m[3] + m[4], m[3] - m[4]
                    y.append([(m[0] + s1) + s2, PA * d1 + PB * d2, A2 * s1 + B2 * s2,
                              ((PA * A2) * d1 + m[5]) + (PB * B2) * d2])
                for r in range(4):
                    ye = pltpu.bitcast(y[0][r].astype(BF16), U32)
                    yo = pltpu.bitcast(y[1][r].astype(BF16), U32)
                    hv = [jnp.where(lo, ye, pltpu.roll(yo, 64, 1)), jnp.where(lo, pltpu.roll(ye, 64, 1), yo)]
                    for j in range(2):
                        l0 = 256 * q + 128 * j
                        o_ref[4 * par + r, :, l0:l0 + 128] = pltpu.bitcast(
                            jnp.take_along_axis(hv[j], idx_in, axis=1), BF16)

    @pl.when(i == 0)
    def _():
        first = pltpu.make_async_copy(x_hbm.at[pl.ds(0, 5)], xb.at[1, pl.ds(3, 5)], sem.at[1])
        first.start()
        full_copy(0, 0).start()
        eye = (jax.lax.broadcasted_iota(jnp.int32, (C, C), 0)
               == jax.lax.broadcasted_iota(jnp.int32, (C, C), 1)).astype(BF16)
        wt = [[jax.lax.dot_general(eye, w_ref[r, s], (((1,), (1,)), ((), ())),
                                   preferred_element_type=F32) for s in range(3)] for r in range(3)]
        for a in range(6):
            ga = [sum(float(GH[a, r]) * wt[r][s] for r in range(3) if GH[a, r] != 0) for s in range(3)]
            u = [sum(float(GW[b, s]) * ga[s] for s in range(3) if GW[b, s] != 0) for b in range(4)]
            u[3] = -u[3]
            for b in range(4):
                ut[a, b] = u[b][:, :128].astype(BF16)
            ut[a, 4] = jnp.concatenate([u[0][:, 128:], u[1][:, 128:]], 1).astype(BF16)
            ut[a, 5] = jnp.concatenate([u[1][:, 128:], u[3][:, 128:]], 1).astype(BF16)
            ut[a, 6] = jnp.concatenate([u[2][:, 128:], u[2][:, 128:]], 1).astype(BF16)
        first.wait()
        wr[2] = jnp.zeros(wr.shape[1:], F32)

        def body(sl, _):
            wstage(1, sl)
        jax.lax.fori_loop(3, 8, body, None)
        for b in range(4):
            hstage(0, (2, 3, 4, 5, 6, 7), b)

    s = i % 2

    @pl.when(i < n - 1)
    def _():
        full_copy(i, s).wait()

    @pl.when(i == n - 1)
    def _():
        last_copy(s).wait()
        xb[s, 3:8] = jnp.zeros((5, C, W), BF16)

    @pl.when(i < n - 2)
    def _():
        full_copy(i + 1, 1 - s).start()

    @pl.when(i == n - 2)
    def _():
        last_copy(1 - s).start()

    for par in range(2):
        slots = (6, 7, 0, 1, 2, 3) if par == 0 else (2, 3, 4, 5, 6, 7)
        for a in range(6):
            mm(par, a)
            if a == 0:
                wstage(s, 4 * par)
                wstage(s, 4 * par + 1)
            elif a == 1:
                wstage(s, 4 * par + 2)
                wstage(s, 4 * par + 3)
            else:
                hstage(1 - par, slots, a - 2)
            if par == 1 and a == 0:
                ostage(0)
    ostage(1)


@jax.jit
def pallas_standalone__winograd__vision_kernel(x, w):
    N, H, Wd, Cc = x.shape
    assert N == 1 and Wd == W and Cc == C and H % 8 == 0 and w.shape == (3, 3, C, C)
    xt = jnp.transpose(x, (0, 1, 3, 2)).reshape(H, C, W)
    out = pl.pallas_call(
        _kernel,
        grid=(H // 8,),
        in_specs=[pl.BlockSpec(memory_space=pl.ANY),
                  pl.BlockSpec((3, 3, C, C), lambda i: (0, 0, 0, 0))],
        out_specs=pl.BlockSpec((8, C, W), lambda i: (i, 0, 0)),
        out_shape=jax.ShapeDtypeStruct((H, C, W), x.dtype),
        scratch_shapes=[
            pltpu.VMEM((2, 8, C, W), BF16),
            pltpu.SemaphoreType.DMA((2,)),
            pltpu.VMEM((6, 7, C, 128), BF16),
            pltpu.VMEM((8, 4, C, P), F32),
            pltpu.VMEM((2, 6, 4, 128, P), BF16),
            pltpu.VMEM((2, 6, 256, P), BF16),
            pltpu.VMEM((2, 6, 2, C, P), F32),
        ],
        compiler_params=pltpu.CompilerParams(
            dimension_semantics=("arbitrary",), vmem_limit_bytes=64 * 1024 * 1024),
    )(xt, w)
    return jnp.transpose(out.reshape(1, H, C, W), (0, 1, 3, 2))
```

```python
import numpy as np
import jax
import jax.numpy as jnp
import jax.experimental.pallas as pl
import jax.experimental.pallas.tpu as pltpu

PA, PB = 1.0, 2.0
_pts = [0.0, PA, -PA, PB, -PB]
GH = np.zeros((6, 3))
for _i, _p in enumerate(_pts):
    GH[_i] = np.array([1.0, _p, _p * _p]) / np.prod([_p - q for q in _pts if q != _p])
GH[5, 2] = 1.0
GW = np.array([[1.0, 0, 0], [0.5, 0.5, 0.5], [0.5, -0.5, 0.5], [0, 0, 1.0]])
A2, B2 = PA * PA, PB * PB
F32, BF16, U32 = jnp.float32, jnp.bfloat16, jnp.uint32
C = 192
W = 512
P = W // 2


def _dot(a, b):
    return jnp.dot(a, b, preferred_element_type=F32)


def _kernel(x_hbm, w_ref, o_ref, xb, sem, ut, wr, vm, vr, ys):
    i = pl.program_id(0)
    n = pl.num_programs(0)
    H = x_hbm.shape[0]

    def full_copy(j, s):
        return pltpu.make_async_copy(x_hbm.at[pl.ds(8 * j + 5, 8)], xb.at[s], sem.at[s])

    def last_copy(s):
        return pltpu.make_async_copy(x_hbm.at[pl.ds(H - 3, 3)], xb.at[s, pl.ds(0, 3)], sem.at[s])

    lane = jax.lax.broadcasted_iota(jnp.int32, (96, 128), 1)
    lo = lane < 64
    idx_de = jnp.where(lo, 2 * lane, 2 * lane - 127)
    idx_in = (lane >> 1) + 64 * (lane & 1)
    zero = jnp.zeros((96, 128), U32)
    bf = lambda u: pltpu.bitcast(u, BF16)
    pk = lambda v: pltpu.bitcast(v.astype(BF16), U32)
    f32 = lambda u: jnp.concatenate([pltpu.unpack_elementwise(
        u, index=k, packed_dtype=BF16, unpacked_dtype=F32) for k in range(2)], 0)
    pke = lambda a, b: pltpu.pack_elementwise([a, b], packed_dtype=BF16)

    def wstage(s, slot):
        if True:
            g = [jnp.take_along_axis(
                pltpu.bitcast(xb[s, slot, :, 128 * j:128 * j + 128], U32), idx_de, axis=1)
                for j in range(4)]
            r = [pltpu.roll(t, 64, 1) for t in g]
            E = [jnp.where(lo, g[2 * q], r[2 * q + 1]) for q in range(2)]
            O = [jnp.where(lo, r[2 * q], g[2 * q + 1]) for q in range(2)]
            Or = [pltpu.roll(t, 1, 1) for t in O]
            Er = [pltpu.roll(t, 127, 1) for t in E]
            Os = [jnp.where(lane == 0, zero, Or[0]), jnp.where(lane == 0, Or[0], Or[1])]
            Es = [jnp.where(lane == 127, Er[1], Er[0]), jnp.where(lane == 127, zero, Er[1])]
            for q in range(2):
                e, o = f32(E[q]), f32(O[q])
                sl = (slice(None), slice(128 * q, 128 * q + 128))
                wr[(slot, 0) + sl] = f32(Os[q]) - o
                wr[(slot, 1) + sl] = e + o
                wr[(slot, 2) + sl] = o - e
                wr[(slot, 3) + sl] = e - f32(Es[q])

    remoff = {0: 0, 1: 64, 3: 128, 2: 192}

    def hstage(par, slots, b):
        for c in range(0, C, 16):
            for q in range(2):
                ls = slice(128 * q, 128 * q + 128)
                d = [jnp.concatenate([wr[sl, b, h + c // 2:h + c // 2 + 8, ls] for h in (0, 96)], 0)
                     for sl in slots]
                t1 = d[4] - 4.0 * d[2]
                t2 = d[3] - 4.0 * d[1]
                t3 = d[4] - d[2]
                t4 = 2.0 * (d[3] - d[1])
                v = [4.0 * (d[0] - d[2]) + t3, t1 + t2, t1 - t2, t3 + t4, t3 - t4,
                     (d[5] - d[3]) - (t4 + t4)]
                for a in range(6):
                    if c < 128:
                        vm[par, a, b, c // 2:c // 2 + 8, ls] = pke(v[a][:8], v[a][8:])
                    else:
                        r0 = (remoff[b] + c - 128) // 2
                        vr[par, a, r0:r0 + 8, ls] = pke(v[a][:8], v[a][8:])

    def mm(par, a):
        m1 = _dot(bf(ut[a, 1]), bf(vm[par, a, 1]))
        m2 = _dot(bf(ut[a, 2]), bf(vm[par, a, 2])) + _dot(bf(ut[a, 6])[:, :64], bf(vr[par, a, 96:128]))
        ye = _dot(bf(ut[a, 0]), bf(vm[par, a, 0])) + _dot(bf(ut[a, 4]), bf(vr[par, a, 0:64]))
        ys[par, a, 0] = (m1 + m2) + ye
        yo = _dot(bf(ut[a, 3]), bf(vm[par, a, 3])) + _dot(bf(ut[a, 5]), bf(vr[par, a, 32:96]))
        ys[par, a, 1] = (m1 - m2) + yo

    def ostage(par):
        if True:
            for q in range(2):
                y = []
                for e in range(2):
                    m = [ys[par, a, e, :, 128 * q:128 * q + 128] for a in range(6)]
                    s1, d1, s2, d2 = m[1] + m[2], m[1] - m[2], m[3] + m[4], m[3] - m[4]
                    y.append([(m[0] + s1) + s2, d1 + PB * d2, s1 + B2 * s2,
                              (d1 + m[5]) + (PB * B2) * d2])
                for r in range(4):
                    ye = pke(y[0][r][:96], y[0][r][96:])
                    yo = pke(y[1][r][:96], y[1][r][96:])
                    hv = [jnp.where(lo, ye, pltpu.roll(yo, 64, 1)), jnp.where(lo, pltpu.roll(ye, 64, 1), yo)]
                    for j in range(2):
                        l0 = 256 * q + 128 * j
                        o_ref[4 * par + r, :, l0:l0 + 128] = pltpu.bitcast(
                            jnp.take_along_axis(hv[j], idx_in, axis=1), BF16)

    @pl.when(i == 0)
    def _():
        first = pltpu.make_async_copy(x_hbm.at[pl.ds(0, 5)], xb.at[1, pl.ds(3, 5)], sem.at[1])
        first.start()
        full_copy(0, 0).start()
        row = jax.lax.broadcasted_iota(jnp.int32, (C, C), 0)
        eye = (row % 96 * 2 + row // 96
               == jax.lax.broadcasted_iota(jnp.int32, (C, C), 1)).astype(BF16)
        wt = [[jax.lax.dot_general(eye, w_ref[r, s], (((1,), (1,)), ((), ())),
                                   preferred_element_type=F32) for s in range(3)] for r in range(3)]
        for a in range(6):
            ga = [sum(float(GH[a, r]) * wt[r][s] for r in range(3) if GH[a, r] != 0) for s in range(3)]
            u = [sum(float(GW[b, s]) * ga[s] for s in range(3) if GW[b, s] != 0) for b in range(4)]
            u[3] = -u[3]
            for b in range(4):
                ut[a, b] = pk(u[b][:, :128])
            ut[a, 4] = pk(jnp.concatenate([u[0][:, 128:], u[1][:, 128:]], 1))
            ut[a, 5] = pk(jnp.concatenate([u[1][:, 128:], u[3][:, 128:]], 1))
            ut[a, 6] = pk(jnp.concatenate([u[2][:, 128:], u[2][:, 128:]], 1))
        first.wait()
        wr[2] = jnp.zeros(wr.shape[1:], F32)

        def body(sl, _):
            wstage(1, sl)
        jax.lax.fori_loop(3, 8, body, None)
        for b in range(4):
            hstage(0, (2, 3, 4, 5, 6, 7), b)

    s = i % 2

    @pl.when(i < n - 1)
    def _():
        full_copy(i, s).wait()

    @pl.when(i == n - 1)
    def _():
        last_copy(s).wait()
        xb[s, 3:8] = jnp.zeros((5, C, W), BF16)

    @pl.when(i < n - 2)
    def _():
        full_copy(i + 1, 1 - s).start()

    @pl.when(i == n - 2)
    def _():
        last_copy(1 - s).start()

    for par in range(2):
        slots = (6, 7, 0, 1, 2, 3) if par == 0 else (2, 3, 4, 5, 6, 7)
        for a in range(6):
            mm(par, a)
            if a == 0:
                wstage(s, 4 * par)
                wstage(s, 4 * par + 1)
            elif a == 1:
                wstage(s, 4 * par + 2)
                wstage(s, 4 * par + 3)
            else:
                hstage(1 - par, slots, a - 2)
            if par == 1 and a == 0:
                ostage(0)
    ostage(1)


@jax.jit
def pallas_standalone__winograd__vision_kernel(x, w):
    N, H, Wd, Cc = x.shape
    assert N == 1 and Wd == W and Cc == C and H % 8 == 0 and w.shape == (3, 3, C, C)
    xt = jnp.transpose(x, (0, 1, 3, 2)).reshape(H, C, W)
    out = pl.pallas_call(
        _kernel,
        grid=(H // 8,),
        in_specs=[pl.BlockSpec(memory_space=pl.ANY),
                  pl.BlockSpec((3, 3, C, C), lambda i: (0, 0, 0, 0))],
        out_specs=pl.BlockSpec((8, C, W), lambda i: (i, 0, 0)),
        out_shape=jax.ShapeDtypeStruct((H, C, W), x.dtype),
        scratch_shapes=[
            pltpu.VMEM((2, 8, C, W), BF16),
            pltpu.SemaphoreType.DMA((2,)),
            pltpu.VMEM((6, 7, C // 2, 128), U32),
            pltpu.VMEM((8, 4, C, P), F32),
            pltpu.VMEM((2, 6, 4, 64, P), U32),
            pltpu.VMEM((2, 6, 128, P), U32),
            pltpu.VMEM((2, 6, 2, C, P), F32),
        ],
        compiler_params=pltpu.CompilerParams(
            dimension_semantics=("arbitrary",), vmem_limit_bytes=64 * 1024 * 1024),
    )(xt, w)
    return jnp.transpose(out.reshape(1, H, C, W), (0, 1, 3, 2))
```

```python
import numpy as np
import jax
import jax.numpy as jnp
import jax.experimental.pallas as pl
import jax.experimental.pallas.tpu as pltpu

PA, PB = 1.0, 2.0
_pts = [0.0, PA, -PA, PB, -PB]
GH = np.zeros((6, 3))
for _i, _p in enumerate(_pts):
    GH[_i] = np.array([1.0, _p, _p * _p]) / np.prod([_p - q for q in _pts if q != _p])
GH[5, 2] = 1.0
GW = np.array([[1.0, 0, 0], [0.5, 0.5, 0.5], [0.5, -0.5, 0.5], [0, 0, 1.0]])
A2, B2 = PA * PA, PB * PB
F32, BF16, U32 = jnp.float32, jnp.bfloat16, jnp.uint32
C = 192
W = 512
P = W // 2


def _dot(a, b):
    return jnp.dot(a, b, preferred_element_type=F32)


def _kernel(x_hbm, w_ref, o_ref, xb, sem, ut, wr, vm, vr, ys, yp):
    i = pl.program_id(0)
    n = pl.num_programs(0)
    H = x_hbm.shape[0]

    def full_copy(j, s):
        return pltpu.make_async_copy(x_hbm.at[pl.ds(8 * j + 5, 8)], xb.at[s], sem.at[s])

    def last_copy(s):
        return pltpu.make_async_copy(x_hbm.at[pl.ds(H - 3, 3)], xb.at[s, pl.ds(0, 3)], sem.at[s])

    lane = jax.lax.broadcasted_iota(jnp.int32, (96, 128), 1)
    lo = lane < 64
    idx_de = jnp.where(lo, 2 * lane, 2 * lane - 127)
    idx_in = (lane >> 1) + 64 * (lane & 1)
    zero = jnp.zeros((96, 128), U32)
    bf = lambda u: pltpu.bitcast(u, BF16)
    pk = lambda v: pltpu.bitcast(v.astype(BF16), U32)
    f32 = lambda u: jnp.concatenate([pltpu.unpack_elementwise(
        u, index=k, packed_dtype=BF16, unpacked_dtype=F32) for k in range(2)], 0)
    pke = lambda a, b: pltpu.pack_elementwise([a, b], packed_dtype=BF16)

    def wstage(s, slot):
        if True:
            g = [jnp.take_along_axis(
                pltpu.bitcast(xb[s, slot, :, 128 * j:128 * j + 128], U32), idx_de, axis=1)
                for j in range(4)]
            r = [pltpu.roll(t, 64, 1) for t in g]
            E = [jnp.where(lo, g[2 * q], r[2 * q + 1]) for q in range(2)]
            O = [jnp.where(lo, r[2 * q], g[2 * q + 1]) for q in range(2)]
            Or = [pltpu.roll(t, 1, 1) for t in O]
            Er = [pltpu.roll(t, 127, 1) for t in E]
            Os = [jnp.where(lane == 0, zero, Or[0]), jnp.where(lane == 0, Or[0], Or[1])]
            Es = [jnp.where(lane == 127, Er[1], Er[0]), jnp.where(lane == 127, zero, Er[1])]
            for q in range(2):
                e, o = f32(E[q]), f32(O[q])
                sl = (slice(None), slice(128 * q, 128 * q + 128))
                wr[(slot, 0) + sl] = f32(Os[q]) - o
                wr[(slot, 1) + sl] = e + o
                wr[(slot, 2) + sl] = o - e
                wr[(slot, 3) + sl] = e - f32(Es[q])

    remoff = {0: 0, 1: 64, 3: 128, 2: 192}

    def hstage(par, slots, b):
        for c in range(0, C, 16):
            for q in range(2):
                ls = slice(128 * q, 128 * q + 128)
                d = [jnp.concatenate([wr[sl, b, h + c // 2:h + c // 2 + 8, ls] for h in (0, 96)], 0)
                     for sl in slots]
                t1 = d[4] - 4.0 * d[2]
                t2 = d[3] - 4.0 * d[1]
                t3 = d[4] - d[2]
                t4 = 2.0 * (d[3] - d[1])
                v = [4.0 * (d[0] - d[2]) + t3, t1 + t2, t1 - t2, t3 + t4, t3 - t4,
                     (d[5] - d[3]) - (t4 + t4)]
                for a in range(6):
                    if c < 128:
                        vm[par, a, b, c // 2:c // 2 + 8, ls] = pke(v[a][:8], v[a][8:])
                    else:
                        r0 = (remoff[b] + c - 128) // 2
                        vr[par, a, r0:r0 + 8, ls] = pke(v[a][:8], v[a][8:])

    def mm(par, a):
        m1 = _dot(bf(ut[a, 1]), bf(vm[par, a, 1]))
        m2 = _dot(bf(ut[a, 2]), bf(vm[par, a, 2])) + _dot(bf(ut[a, 6])[:, :64], bf(vr[par, a, 96:128]))
        ye = _dot(bf(ut[a, 0]), bf(vm[par, a, 0])) + _dot(bf(ut[a, 4]), bf(vr[par, a, 0:64]))
        ys[par, a, 0] = (m1 + m2) + ye
        yo = _dot(bf(ut[a, 3]), bf(vm[par, a, 3])) + _dot(bf(ut[a, 5]), bf(vr[par, a, 32:96]))
        ys[par, a, 1] = (m1 - m2) + yo

    def ostage(par):
        for c in range(0, 96, 8):
            for q in range(2):
                y = []
                for e in range(2):
                    m = [jnp.concatenate([ys[par, a, e, h + c:h + c + 8, 128 * q:128 * q + 128]
                                          for h in (0, 96)], 0) for a in range(6)]
                    s1, d1, s2, d2 = m[1] + m[2], m[1] - m[2], m[3] + m[4], m[3] - m[4]
                    y.append([(m[0] + s1) + s2, d1 + PB * d2, s1 + B2 * s2,
                              (d1 + m[5]) + (PB * B2) * d2])
                for r in range(4):
                    for e in range(2):
                        yp[r, e, c:c + 8, 128 * q:128 * q + 128] = pke(y[e][r][:8], y[e][r][8:])
        for q in range(2):
            for r in range(4):
                if True:
                    ye, yo = (yp[r, e, :, 128 * q:128 * q + 128] for e in range(2))
                    hv = [jnp.where(lo, ye, pltpu.roll(yo, 64, 1)), jnp.where(lo, pltpu.roll(ye, 64, 1), yo)]
                    for j in range(2):
                        l0 = 256 * q + 128 * j
                        o_ref[4 * par + r, :, l0:l0 + 128] = pltpu.bitcast(
                            jnp.take_along_axis(hv[j], idx_in, axis=1), BF16)

    @pl.when(i == 0)
    def _():
        first = pltpu.make_async_copy(x_hbm.at[pl.ds(0, 5)], xb.at[1, pl.ds(3, 5)], sem.at[1])
        first.start()
        full_copy(0, 0).start()
        row = jax.lax.broadcasted_iota(jnp.int32, (C, C), 0)
        eye = (row % 96 * 2 + row // 96
               == jax.lax.broadcasted_iota(jnp.int32, (C, C), 1)).astype(BF16)
        wt = [[jax.lax.dot_general(eye, w_ref[r, s], (((1,), (1,)), ((), ())),
                                   preferred_element_type=F32) for s in range(3)] for r in range(3)]
        for a in range(6):
            ga = [sum(float(GH[a, r]) * wt[r][s] for r in range(3) if GH[a, r] != 0) for s in range(3)]
            u = [sum(float(GW[b, s]) * ga[s] for s in range(3) if GW[b, s] != 0) for b in range(4)]
            u[3] = -u[3]
            for b in range(4):
                ut[a, b] = pk(u[b][:, :128])
            ut[a, 4] = pk(jnp.concatenate([u[0][:, 128:], u[1][:, 128:]], 1))
            ut[a, 5] = pk(jnp.concatenate([u[1][:, 128:], u[3][:, 128:]], 1))
            ut[a, 6] = pk(jnp.concatenate([u[2][:, 128:], u[2][:, 128:]], 1))
        first.wait()
        wr[2] = jnp.zeros(wr.shape[1:], F32)

        def body(sl, _):
            wstage(1, sl)
        jax.lax.fori_loop(3, 8, body, None)
        for b in range(4):
            hstage(0, (2, 3, 4, 5, 6, 7), b)

    s = i % 2

    @pl.when(i < n - 1)
    def _():
        full_copy(i, s).wait()

    @pl.when(i == n - 1)
    def _():
        last_copy(s).wait()
        xb[s, 3:8] = jnp.zeros((5, C, W), BF16)

    @pl.when(i < n - 2)
    def _():
        full_copy(i + 1, 1 - s).start()

    @pl.when(i == n - 2)
    def _():
        last_copy(1 - s).start()

    for par in range(2):
        slots = (6, 7, 0, 1, 2, 3) if par == 0 else (2, 3, 4, 5, 6, 7)
        for a in range(6):
            mm(par, a)
            if a == 0:
                wstage(s, 4 * par)
                wstage(s, 4 * par + 1)
            elif a == 1:
                wstage(s, 4 * par + 2)
                wstage(s, 4 * par + 3)
            else:
                hstage(1 - par, slots, a - 2)
            if par == 1 and a == 1:
                ostage(0)
    ostage(1)


@jax.jit
def pallas_standalone__winograd__vision_kernel(x, w):
    N, H, Wd, Cc = x.shape
    assert N == 1 and Wd == W and Cc == C and H % 8 == 0 and w.shape == (3, 3, C, C)
    xt = jnp.transpose(x, (0, 1, 3, 2)).reshape(H, C, W)
    out = pl.pallas_call(
        _kernel,
        grid=(H // 8,),
        in_specs=[pl.BlockSpec(memory_space=pl.ANY),
                  pl.BlockSpec((3, 3, C, C), lambda i: (0, 0, 0, 0))],
        out_specs=pl.BlockSpec((8, C, W), lambda i: (i, 0, 0)),
        out_shape=jax.ShapeDtypeStruct((H, C, W), x.dtype),
        scratch_shapes=[
            pltpu.VMEM((2, 8, C, W), BF16),
            pltpu.SemaphoreType.DMA((2,)),
            pltpu.VMEM((6, 7, C // 2, 128), U32),
            pltpu.VMEM((8, 4, C, P), F32),
            pltpu.VMEM((2, 6, 4, 64, P), U32),
            pltpu.VMEM((2, 6, 128, P), U32),
            pltpu.VMEM((2, 6, 2, C, P), F32),
            pltpu.VMEM((4, 2, C // 2, P), U32),
        ],
        compiler_params=pltpu.CompilerParams(
            dimension_semantics=("arbitrary",), vmem_limit_bytes=64 * 1024 * 1024),
    )(xt, w)
    return jnp.transpose(out.reshape(1, H, C, W), (0, 1, 3, 2))
```
